```python
import os as _os
_os.environ.setdefault("JAX_PLATFORMS", "cpu")
import jax
import jax.numpy as jnp

def _softmax(x, axis=-1):
    return jax.nn.softmax(x, axis=axis)
def _gelu(x):
    return jax.nn.gelu(x, approximate=True)
def _silu(x):
    return jax.nn.silu(x)
def _sigmoid(x):
    return jax.nn.sigmoid(x)
def _layernorm(x, axis=-1, eps=1e-5):
    m = jnp.mean(x, axis=axis, keepdims=True)
    v = jnp.var(x, axis=axis, keepdims=True)
    return (x - m) / jnp.sqrt(v + eps)
def _scatter_add(tgt, idx, src, axis=0):
    return tgt.at[idx].add(src)
def _segment_sum(src, seg, n):
    return jax.ops.segment_sum(src, seg, n)
class _Rng:
    def __init__(self, key):
        self._k = key
    def _next(self):
        self._k, sub = jax.random.split(self._k)
        return sub
    def normal(self, shape):
        return jax.random.normal(self._next(), shape, dtype=jnp.bfloat16)
    def randint(self, lo, hi, shape):
        return jax.random.randint(self._next(), shape, lo, hi, dtype=jnp.int32)
    def uniform(self, shape, lo=0.0, hi=1.0):
        return jax.random.uniform(self._next(), shape, jnp.bfloat16, lo, hi)
    def permutation(self, n):
        return jax.random.permutation(self._next(), n)


kernel_name = 'gated_mix__ssm_conv_s5__glu_gated_geglu__prompt'

def setup_inputs():
    _rng = _Rng(jax.random.key(int.from_bytes(__import__("os").urandom(4), "little")))
    _w = (lambda a: (lambda t: t.astype(jnp.bfloat16) if jnp.issubdtype(t.dtype, jnp.floating) else t)(jnp.asarray(a)))
    def _A_setup():
        B, S, D = 1, 2048, 1024
        P = D
        Lambda_re = -0.5 * jnp.exp((lambda *s: _rng.normal(s) * 0.4)(P))
        Lambda_im = (lambda *s: _rng.normal(s) * 0.4)(P) * 1.0
        B_re = (lambda *s: _rng.normal(s) * 0.4)(P, D) * (D ** -0.5)
        B_im = (lambda *s: _rng.normal(s) * 0.4)(P, D) * (D ** -0.5)
        C_re = (lambda *s: _rng.normal(s) * 0.4)(D, P) * (P ** -0.5)
        C_im = (lambda *s: _rng.normal(s) * 0.4)(D, P) * (P ** -0.5)
        log_dt = (lambda *s: _rng.normal(s) * 0.4)(P) * 0.3 - 2.0
        Dskip = (lambda *s: _rng.normal(s) * 0.4)(D)
        return {
            "x": _w((lambda *s: _rng.normal(s) * 0.05)(B, S, D)),
            "Lambda_re": _w(Lambda_re),
            "Lambda_im": _w(Lambda_im),
            "B_re": _w(B_re),
            "B_im": _w(B_im),
            "C_re": _w(C_re),
            "C_im": _w(C_im),
            "log_dt": _w(log_dt),
            "Dskip": _w(Dskip),
        }
    _A_in = _A_setup()

    def _B_setup():
        B, S, Dm, Df = 1, 2048, 1024, 3584
        return {
            "x": _w((lambda *s: _rng.normal(s) * 0.05)(B, S, Dm)),
            "w_gate": _w((lambda *s: _rng.normal(s) * 1.6)(Dm, Df) * (Dm ** -0.5)),
            "w_up": _w((lambda *s: _rng.normal(s) * 1.6)(Dm, Df) * (Dm ** -0.5)),
            "w_down": _w((lambda *s: _rng.normal(s) * 1.6)(Df, Dm) * (Df ** -0.5)),
        }
    _B_in = _B_setup()

    return {
        "A_x": _A_in["x"],
        "A_Lambda_re": _A_in["Lambda_re"],
        "A_Lambda_im": _A_in["Lambda_im"],
        "A_B_re": _A_in["B_re"],
        "A_B_im": _A_in["B_im"],
        "A_C_re": _A_in["C_re"],
        "A_C_im": _A_in["C_im"],
        "A_log_dt": _A_in["log_dt"],
        "A_Dskip": _A_in["Dskip"],
        "B_x": _B_in["x"],
        "B_w_gate": _B_in["w_gate"],
        "B_w_up": _B_in["w_up"],
        "B_w_down": _B_in["w_down"],
        "gate_w": _w((lambda *s: _rng.normal(s) * 0.05)(1024) * 16.0),
    }

def reference(A_x, A_Lambda_re, A_Lambda_im, A_B_re, A_B_im, A_C_re, A_C_im, A_log_dt, A_Dskip, B_x, B_w_gate, B_w_up, B_w_down, gate_w):
    def _A_ref(x, Lambda_re, Lambda_im, B_re, B_im, C_re, C_im, log_dt, Dskip):
        Bsz, L, H = x.shape
        Lam = Lambda_re + 1j * Lambda_im
        Bmat = B_re + 1j * B_im
        Cmat = C_re + 1j * C_im
        dt = jnp.exp(log_dt)
        Lam_bar = jnp.exp(dt * Lam)
        B_bar = ((Lam_bar - 1.0) / Lam)[:, None] * Bmat
        Bu = jnp.einsum("bld,pd->blp", x + 0j, B_bar)
        h = jnp.zeros_like(Bu[:, 0, :])
        hs = []
        for t in range(L):
            h = Lam_bar[None, :] * h + Bu[:, t, :]
            hs.append(h)
        hseq = jnp.stack(hs, 1)
        y = 2.0 * jnp.einsum("blp,dp->bld", hseq, Cmat).real + x * Dskip[None, None, :]
        return y

    def _B_ref(x, w_gate, w_up, w_down):
        g = jnp.einsum("bsd,df->bsf", x, w_gate)
        u = jnp.einsum("bsd,df->bsf", x, w_up)
        h = _gelu(g) * u
        return jnp.einsum("bsf,fd->bsd", h, w_down)

    x = A_x
    g = _sigmoid((x * gate_w).sum(-1, keepdims=True))
    a = _A_ref(x, A_Lambda_re, A_Lambda_im, A_B_re, A_B_im, A_C_re, A_C_im, A_log_dt, A_Dskip)
    b = _B_ref(x, B_w_gate, B_w_up, B_w_down)
    return g * a + (1 - g) * b
```

```python
import jax
import jax.numpy as jnp
import jax.experimental.pallas as pl
import jax.experimental.pallas.tpu as pltpu

L = 2048
D = 1024
P = 1024
DF = 3584
T = 512
S = T // 8
FC = 512
NF = DF // FC


def _gelu_tanh(x):
    c = 0.7978845608028654
    return 0.5 * x * (1.0 + jnp.tanh(c * (x + 0.044715 * (x * x * x))))


def _kernel(x_ref, lre_ref, lim_ref, bre_ref, bim_ref, cre_ref, cim_ref, ldt_ref, dsk_ref,
            wg_ref, wu_ref, wd_ref, gw_ref, o_ref,
            bbar_ref, ccat_ref, lam_ref, pow_ref, carry_ref, bu_ref, hb_ref):
    f32 = jnp.float32
    bf16 = jnp.bfloat16
    step = pl.program_id(0)

    @pl.when(step == 0)
    def _init():
        lam_re = lre_ref[...].astype(f32)
        lam_im = lim_ref[...].astype(f32)
        dt = jnp.exp(ldt_ref[...].astype(f32)).astype(bf16).astype(f32)
        a = dt * lam_re
        b = dt * lam_im
        ea = jnp.exp(a)
        lb_re = ea * jnp.cos(b)
        lb_im = ea * jnp.sin(b)
        nr = lb_re - 1.0
        ni = lb_im
        den = lam_re * lam_re + lam_im * lam_im
        cf_re = (nr * lam_re + ni * lam_im) / den
        cf_im = (ni * lam_re - nr * lam_im) / den
        bt_re = bre_ref[...].astype(f32).T
        bt_im = bim_ref[...].astype(f32).T
        bbar_ref[:, :P] = (cf_re * bt_re - cf_im * bt_im).astype(bf16)
        bbar_ref[:, P:] = (cf_re * bt_im + cf_im * bt_re).astype(bf16)
        ccat_ref[:P, :] = (2.0 * cre_ref[...].astype(f32)).T.astype(bf16)
        ccat_ref[P:, :] = (-2.0 * cim_ref[...].astype(f32)).T.astype(bf16)
        lam_ref[:, :P] = jnp.broadcast_to(lb_re, (8, P))
        lam_ref[:, P:] = jnp.broadcast_to(lb_im, (8, P))
        pow_ref[0:1, :P] = lb_re
        pow_ref[0:1, P:] = lb_im

        def pbody(k, c):
            pr, pi = c
            nr_ = pr * lb_re - pi * lb_im
            ni_ = pr * lb_im + pi * lb_re
            pow_ref[pl.ds(k, 1), :P] = nr_
            pow_ref[pl.ds(k, 1), P:] = ni_
            return nr_, ni_
        jax.lax.fori_loop(1, S, pbody, (lb_re, lb_im))
        carry_ref[...] = jnp.zeros(carry_ref.shape, f32)

    xt = x_ref[...]

    bu = jnp.dot(xt, bbar_ref[...], preferred_element_type=f32)
    NG = 2 * P // 128
    for j in range(NG):
        bu_ref[j] = bu[:, j * 128:(j + 1) * 128]
    lr = lam_ref[:, :P]
    li = lam_ref[:, P:]

    def sbody(k, c):
        hr, hi = c
        ur = jnp.concatenate([bu_ref[j, pl.ds(k, 8, stride=S), :] for j in range(NG // 2)], axis=1)
        ui = jnp.concatenate([bu_ref[NG // 2 + j, pl.ds(k, 8, stride=S), :] for j in range(NG // 2)], axis=1)
        nr_ = lr * hr - li * hi + ur
        ni_ = lr * hi + li * hr + ui
        for j in range(NG // 2):
            bu_ref[j, pl.ds(k, 8, stride=S), :] = nr_[:, j * 128:(j + 1) * 128]
            bu_ref[NG // 2 + j, pl.ds(k, 8, stride=S), :] = ni_[:, j * 128:(j + 1) * 128]
        return nr_, ni_
    zeros8 = jnp.zeros((8, P), f32)
    fr, fi = jax.lax.fori_loop(0, S, sbody, (zeros8, zeros8))

    ps_re = pow_ref[S - 1:S, :P]
    ps_im = pow_ref[S - 1:S, P:]
    cr = carry_ref[0:1, :P]
    ci = carry_ref[0:1, P:]
    pw_re = pow_ref[:, :P]
    pw_im = pow_ref[:, P:]
    for i in range(8):
        rows = slice(i * S, (i + 1) * S)
        br = jnp.concatenate([bu_ref[j, rows, :] for j in range(NG // 2)], axis=1)
        bi = jnp.concatenate([bu_ref[NG // 2 + j, rows, :] for j in range(NG // 2)], axis=1)
        hr = br + (pw_re * cr - pw_im * ci)
        hi = bi + (pw_re * ci + pw_im * cr)
        hb_ref[rows, :P] = hr.astype(bf16)
        hb_ref[rows, P:] = hi.astype(bf16)
        ncr = fr[i:i + 1, :] + (ps_re * cr - ps_im * ci)
        nci = fi[i:i + 1, :] + (ps_re * ci + ps_im * cr)
        cr, ci = ncr, nci
    carry_ref[0:1, :P] = cr
    carry_ref[0:1, P:] = ci

    ya = jnp.dot(hb_ref[...], ccat_ref[...], preferred_element_type=f32)
    ya = ya + (xt * dsk_ref[...]).astype(f32)

    acc = jnp.zeros((T, D), f32)
    for c in range(NF):
        cs = slice(c * FC, (c + 1) * FC)
        g = jnp.dot(xt, wg_ref[:, cs], preferred_element_type=f32).astype(bf16).astype(f32)
        u = jnp.dot(xt, wu_ref[:, cs], preferred_element_type=f32).astype(bf16).astype(f32)
        hh = (_gelu_tanh(g).astype(bf16).astype(f32) * u).astype(bf16)
        acc = acc + jnp.dot(hh, wd_ref[cs, :], preferred_element_type=f32)
    yb = acc.astype(bf16)

    s = jnp.sum((xt * gw_ref[...]).astype(f32), axis=-1, keepdims=True)
    gt = jax.nn.sigmoid(s.astype(bf16).astype(f32)).astype(bf16)
    o_ref[...] = gt.astype(f32) * ya + ((1.0 - gt.astype(f32)).astype(bf16) * yb).astype(f32)


@jax.jit
def pallas_gated_mix__ssm_conv_s5__glu_gated_geglu__prompt_kernel(
    A_x, A_Lambda_re, A_Lambda_im, A_B_re, A_B_im, A_C_re, A_C_im, A_log_dt, A_Dskip,
    B_x, B_w_gate, B_w_up, B_w_down, gate_w,
):
    x2 = A_x.reshape(L, D)
    row = lambda v: v.reshape(1, -1)
    const = lambda shape: pl.BlockSpec(shape, lambda i: (0, 0), pipeline_mode=pl.Buffered(1))
    out = pl.pallas_call(
        _kernel,
        grid=(L // T,),
        in_specs=[
            pl.BlockSpec((T, D), lambda i: (i, 0)),
            const((1, P)), const((1, P)),
            const((P, D)), const((P, D)),
            const((D, P)), const((D, P)),
            const((1, P)), const((1, D)),
            const((D, DF)), const((D, DF)), const((DF, D)),
            const((1, D)),
        ],
        out_specs=pl.BlockSpec((T, D), lambda i: (i, 0)),
        out_shape=jax.ShapeDtypeStruct((L, D), jnp.float32),
        scratch_shapes=[
            pltpu.VMEM((D, 2 * P), jnp.bfloat16),
            pltpu.VMEM((2 * P, D), jnp.bfloat16),
            pltpu.VMEM((8, 2 * P), jnp.float32),
            pltpu.VMEM((S, 2 * P), jnp.float32),
            pltpu.VMEM((8, 2 * P), jnp.float32),
            pltpu.VMEM((2 * P // 128, T, 128), jnp.float32),
            pltpu.VMEM((T, 2 * P), jnp.bfloat16),
        ],
        compiler_params=pltpu.CompilerParams(
            dimension_semantics=("arbitrary",),
            vmem_limit_bytes=110 * 1024 * 1024,
        ),
    )(x2, row(A_Lambda_re), row(A_Lambda_im), A_B_re, A_B_im, A_C_re, A_C_im,
      row(A_log_dt), row(A_Dskip), B_w_gate, B_w_up, B_w_down, row(gate_w))
    return out.reshape(1, L, D)
```

```python
import jax
import jax.numpy as jnp
import jax.experimental.pallas as pl
import jax.experimental.pallas.tpu as pltpu

L = 2048
D = 1024
P = 1024
DF = 3584
T = 512
NB = T // 8
FC = 512
NF = DF // FC
NGRP = P // 128

NT_DIMS = (((1,), (1,)), ((), ()))


def _gelu_tanh(x):
    c = 0.7978845608028654
    return 0.5 * x * (1.0 + jnp.tanh(c * (x + 0.044715 * (x * x * x))))


def _cmul(ar, ai, br, bi):
    return ar * br - ai * bi, ar * bi + ai * br


def _kernel(x_ref, lre_ref, lim_ref, ldt_ref, dsk_ref, gw_ref,
            bre_hbm, bim_hbm, cre_hbm, cim_hbm, wg_hbm, wu_hbm, wd_hbm,
            o_ref,
            bre_ref, bim_ref, cre_ref, cim_ref, wg_ref, wu_ref, wd_ref,
            tab_ref, carry_ref, h_ref, acc_ref, sems):
    f32 = jnp.float32
    bf16 = jnp.bfloat16
    step = pl.program_id(0)

    def ssm_copies():
        return [pltpu.make_async_copy(bre_hbm, bre_ref, sems.at[0]),
                pltpu.make_async_copy(bim_hbm, bim_ref, sems.at[1])]

    def c_copies():
        return [pltpu.make_async_copy(cre_hbm, cre_ref, sems.at[2]),
                pltpu.make_async_copy(cim_hbm, cim_ref, sems.at[3])]

    def ffn_copies(c):
        cs = pl.ds(c * FC, FC)
        return [pltpu.make_async_copy(wg_hbm.at[:, cs], wg_ref.at[:, cs], sems.at[4 + 3 * c]),
                pltpu.make_async_copy(wu_hbm.at[:, cs], wu_ref.at[:, cs], sems.at[5 + 3 * c]),
                pltpu.make_async_copy(wd_hbm.at[cs, :], wd_ref.at[cs, :], sems.at[6 + 3 * c])]

    @pl.when(step == 0)
    def _init():
        for cp in ssm_copies():
            cp.start()
        for c in range(NF):
            for cp in ffn_copies(c):
                cp.start()
        for cp in c_copies():
            cp.start()
        lam_re = lre_ref[...].astype(f32)
        lam_im = lim_ref[...].astype(f32)
        dt = jnp.exp(ldt_ref[...].astype(f32)).astype(bf16).astype(f32)
        a = dt * lam_re
        b = dt * lam_im
        ea = jnp.exp(a)
        l1r = ea * jnp.cos(b)
        l1i = ea * jnp.sin(b)
        nr = l1r - 1.0
        ni = l1i
        den = lam_re * lam_re + lam_im * lam_im
        cf_re = (nr * lam_re + ni * lam_im) / den
        cf_im = (ni * lam_re - nr * lam_im) / den
        pows = [(l1r, l1i)]
        for _ in range(7):
            pows.append(_cmul(pows[-1][0], pows[-1][1], l1r, l1i))
        rid = jax.lax.broadcasted_iota(jnp.int32, (8, P), 0)
        bc = lambda v: jnp.broadcast_to(v, (8, P))
        tab_ref[0] = bc(cf_re)
        tab_ref[1] = bc(cf_im)
        for n, s in enumerate((1, 2, 4)):
            tab_ref[2 + 2 * n] = jnp.where(rid >= s, bc(pows[s - 1][0]), 0.0)
            tab_ref[3 + 2 * n] = jnp.where(rid >= s, bc(pows[s - 1][1]), 0.0)
        pwr = bc(pows[0][0])
        pwi = bc(pows[0][1])
        for t in range(1, 8):
            pwr = jnp.where(rid == t, bc(pows[t][0]), pwr)
            pwi = jnp.where(rid == t, bc(pows[t][1]), pwi)
        tab_ref[8] = pwr
        tab_ref[9] = pwi
        carry_ref[...] = jnp.zeros(carry_ref.shape, f32)
        for cp in ssm_copies():
            cp.wait()

    xt = x_ref[...]

    h_ref[:, :P] = jax.lax.dot_general(xt, bre_ref[...], NT_DIMS, preferred_element_type=f32)
    h_ref[:, P:] = jax.lax.dot_general(xt, bim_ref[...], NT_DIMS, preferred_element_type=f32)

    def scan_group(j):
        if isinstance(j, int):
            lr = slice(j * 128, (j + 1) * 128)
            li = slice(P + j * 128, P + (j + 1) * 128)
        else:
            lr = pl.ds(pl.multiple_of(j * 128, 128), 128)
            li = pl.ds(pl.multiple_of(P + j * 128, 128), 128)
        tabs = [tab_ref[n, :, lr] for n in range(10)]
        cr = carry_ref[0, :, lr]
        ci = carry_ref[1, :, lr]
        for kb in range(NB):
            rows = slice(kb * 8, kb * 8 + 8)
            hr, hi = _cmul(tabs[0], tabs[1], h_ref[rows, lr], h_ref[rows, li])
            for n, s in enumerate((1, 2, 4)):
                sr = pltpu.roll(hr, s, 0)
                si = pltpu.roll(hi, s, 0)
                dr, di = _cmul(tabs[2 + 2 * n], tabs[3 + 2 * n], sr, si)
                hr = hr + dr
                hi = hi + di
            dr, di = _cmul(tabs[8], tabs[9], cr, ci)
            hr = hr + dr
            hi = hi + di
            cr = jnp.broadcast_to(hr[7:8, :], (8, 128))
            ci = jnp.broadcast_to(hi[7:8, :], (8, 128))
            h_ref[rows, lr] = hr * 2.0
            h_ref[rows, li] = hi * (-2.0)
        carry_ref[0, :, lr] = cr
        carry_ref[1, :, lr] = ci

    scan_group(NGRP - 1)

    def ffn_body(c, _):
        @pl.when(step == 0)
        def _wait():
            for cp in ffn_copies(c):
                cp.wait()
        cs = pl.ds(pl.multiple_of(c * FC, FC), FC)
        g = jnp.dot(xt, wg_ref[:, cs], preferred_element_type=f32).astype(bf16).astype(f32)
        u = jnp.dot(xt, wu_ref[:, cs], preferred_element_type=f32).astype(bf16).astype(f32)
        hh = (_gelu_tanh(g).astype(bf16).astype(f32) * u).astype(bf16)
        part = jnp.dot(hh, wd_ref[cs, :], preferred_element_type=f32)
        acc_ref[...] += part
        scan_group(c)
        return 0
    acc_ref[...] = jnp.zeros((T, D), f32)
    jax.lax.fori_loop(0, NF, ffn_body, 0)
    yb = acc_ref[...].astype(bf16)

    @pl.when(step == 0)
    def _wait_c():
        for cp in c_copies():
            cp.wait()

    hre = h_ref[:, :P].astype(bf16)
    him = h_ref[:, P:].astype(bf16)
    ya = (jax.lax.dot_general(hre, cre_ref[...], NT_DIMS, preferred_element_type=f32)
          + jax.lax.dot_general(him, cim_ref[...], NT_DIMS, preferred_element_type=f32))
    ya = ya + (xt * dsk_ref[...]).astype(f32)

    s = jnp.sum((xt * gw_ref[...]).astype(f32), axis=-1, keepdims=True)
    gt = jax.nn.sigmoid(s.astype(bf16).astype(f32)).astype(bf16)
    o_ref[...] = gt.astype(f32) * ya + ((1.0 - gt.astype(f32)).astype(bf16) * yb).astype(f32)


@jax.jit
def pallas_gated_mix__ssm_conv_s5__glu_gated_geglu__prompt_kernel(
    A_x, A_Lambda_re, A_Lambda_im, A_B_re, A_B_im, A_C_re, A_C_im, A_log_dt, A_Dskip,
    B_x, B_w_gate, B_w_up, B_w_down, gate_w,
):
    x2 = A_x.reshape(L, D)
    row = lambda v: v.reshape(1, -1)
    const = lambda shape: pl.BlockSpec(shape, lambda i: (0, 0))
    hbm = pl.BlockSpec(memory_space=pl.ANY)
    out = pl.pallas_call(
        _kernel,
        grid=(L // T,),
        in_specs=[
            pl.BlockSpec((T, D), lambda i: (i, 0)),
            const((1, P)), const((1, P)), const((1, P)), const((1, D)), const((1, D)),
            hbm, hbm, hbm, hbm, hbm, hbm, hbm,
        ],
        out_specs=pl.BlockSpec((T, D), lambda i: (i, 0)),
        out_shape=jax.ShapeDtypeStruct((L, D), jnp.float32),
        scratch_shapes=[
            pltpu.VMEM((P, D), jnp.bfloat16),
            pltpu.VMEM((P, D), jnp.bfloat16),
            pltpu.VMEM((D, P), jnp.bfloat16),
            pltpu.VMEM((D, P), jnp.bfloat16),
            pltpu.VMEM((D, DF), jnp.bfloat16),
            pltpu.VMEM((D, DF), jnp.bfloat16),
            pltpu.VMEM((DF, D), jnp.bfloat16),
            pltpu.VMEM((10, 8, P), jnp.float32),
            pltpu.VMEM((2, 8, P), jnp.float32),
            pltpu.VMEM((T, 2 * P), jnp.float32),
            pltpu.VMEM((T, D), jnp.float32),
            pltpu.SemaphoreType.DMA((4 + 3 * NF,)),
        ],
        compiler_params=pltpu.CompilerParams(
            dimension_semantics=("arbitrary",),
            vmem_limit_bytes=110 * 1024 * 1024,
        ),
    )(x2, row(A_Lambda_re), row(A_Lambda_im), row(A_log_dt), row(A_Dskip), row(gate_w),
      A_B_re, A_B_im, A_C_re, A_C_im, B_w_gate, B_w_up, B_w_down)
    return out.reshape(1, L, D)
```

```python
import jax
import jax.numpy as jnp
import jax.experimental.pallas as pl
import jax.experimental.pallas.tpu as pltpu

L = 2048
D = 1024
P = 1024
DF = 3584
T = 512
NB = T // 8
FC = 512
NF = DF // FC
NGRP = P // 128
OC = 256
XB = (NB - 1) // NF
assert XB * NF + 1 == NB
BC = 512
NBC = P // BC
NOC = D // OC

NT_DIMS = (((1,), (1,)), ((), ()))


def _gelu_tanh(x):
    c = 0.7978845608028654
    return 0.5 * x * (1.0 + jnp.tanh(c * (x + 0.044715 * (x * x * x))))


def _cmul(ar, ai, br, bi):
    return ar * br - ai * bi, ar * bi + ai * br


def _kernel(x_ref, lre_ref, lim_ref, ldt_ref, dsk_ref, gw_ref,
            bre_hbm, bim_hbm, cre_hbm, cim_hbm, wg_hbm, wu_hbm, wd_hbm,
            o_ref,
            bre_ref, bim_ref, cre_ref, cim_ref, wg_ref, wu_ref, wd_ref,
            tab_ref, carry_ref, h_ref, acc_ref, obuf_ref, gate_ref, sems, osems, bsems):
    f32 = jnp.float32
    bf16 = jnp.bfloat16
    step = pl.program_id(0)

    def ssm_copies(n):
        rs = pl.ds(n * BC, BC)
        return [pltpu.make_async_copy(bre_hbm.at[rs, :], bre_ref.at[rs, :], bsems.at[2 * n]),
                pltpu.make_async_copy(bim_hbm.at[rs, :], bim_ref.at[rs, :], bsems.at[2 * n + 1])]

    def c_copies():
        return [pltpu.make_async_copy(cre_hbm, cre_ref, sems.at[0]),
                pltpu.make_async_copy(cim_hbm, cim_ref, sems.at[1])]

    def ffn_copies(c):
        cs = pl.ds(c * FC, FC)
        return [pltpu.make_async_copy(wg_hbm.at[:, cs], wg_ref.at[:, cs], sems.at[2 + 3 * c]),
                pltpu.make_async_copy(wu_hbm.at[:, cs], wu_ref.at[:, cs], sems.at[3 + 3 * c]),
                pltpu.make_async_copy(wd_hbm.at[cs, :], wd_ref.at[cs, :], sems.at[4 + 3 * c])]

    def out_copy(st, n):
        cols = pl.ds(n * OC, OC)
        rows = pl.ds(pl.multiple_of(st * T, T), T)
        return pltpu.make_async_copy(obuf_ref.at[st % 2, :, cols], o_ref.at[rows, cols],
                                     osems.at[st % 2, n])

    @pl.when(step == 0)
    def _init():
        for n in range(NBC):
            for cp in ssm_copies(n):
                cp.start()
        lam_re = lre_ref[...].astype(f32).reshape(1, P)
        lam_im = lim_ref[...].astype(f32).reshape(1, P)
        dt = jnp.exp(ldt_ref[...].astype(f32).reshape(1, P)).astype(bf16).astype(f32)
        a = dt * lam_re
        b = dt * lam_im
        ea = jnp.exp(a)
        l1r = ea * jnp.cos(b)
        l1i = ea * jnp.sin(b)
        nr = l1r - 1.0
        ni = l1i
        den = lam_re * lam_re + lam_im * lam_im
        cf_re = (nr * lam_re + ni * lam_im) / den
        cf_im = (ni * lam_re - nr * lam_im) / den
        pows = [(l1r, l1i)]
        for _ in range(7):
            pows.append(_cmul(pows[-1][0], pows[-1][1], l1r, l1i))
        rid = jax.lax.broadcasted_iota(jnp.int32, (8, P), 0)
        bc = lambda v: jnp.broadcast_to(v, (8, P))
        tab_ref[0] = bc(cf_re)
        tab_ref[1] = bc(cf_im)
        for n, s in enumerate((1, 2, 4)):
            tab_ref[2 + 2 * n] = jnp.where(rid >= s, bc(pows[s - 1][0]), 0.0)
            tab_ref[3 + 2 * n] = jnp.where(rid >= s, bc(pows[s - 1][1]), 0.0)
        pwr = bc(pows[0][0])
        pwi = bc(pows[0][1])
        for t in range(1, 8):
            pwr = jnp.where(rid == t, bc(pows[t][0]), pwr)
            pwi = jnp.where(rid == t, bc(pows[t][1]), pwi)
        tab_ref[8] = pwr
        tab_ref[9] = pwi
        carry_ref[...] = jnp.zeros(carry_ref.shape, f32)


    def bu_body(n, _):
        @pl.when(step == 0)
        def _wait_b():
            for cp in ssm_copies(n):
                cp.wait()

            @pl.when(n >= NBC - 2)
            def _start_ffn():
                for cp in ffn_copies(jnp.maximum(n - (NBC - 2), 0)):
                    cp.start()
        hrows = pl.ds(pl.multiple_of(n * (T // NBC), T // NBC), T // NBC)
        acc_ref[hrows, :] = jnp.zeros((T // NBC, D), f32)
        sg = jnp.sum((x_ref[hrows, :] * gw_ref[...].reshape(1, D)).astype(f32), axis=-1, keepdims=True)
        gt = jax.nn.sigmoid(sg.astype(bf16).astype(f32)).astype(bf16)
        gate_ref[hrows, :] = jnp.broadcast_to(gt.astype(f32), (T // NBC, 128))
        rs = pl.ds(pl.multiple_of(n * BC, BC), BC)
        ri = pl.ds(pl.multiple_of(P + n * BC, BC), BC)
        h_ref[:, rs] = jax.lax.dot_general(x_ref[...], bre_ref[rs, :], NT_DIMS, preferred_element_type=f32)
        h_ref[:, ri] = jax.lax.dot_general(x_ref[...], bim_ref[rs, :], NT_DIMS, preferred_element_type=f32)
        return 0
    jax.lax.fori_loop(0, NBC, bu_body, 0)

    def scan_group(j, row0=0, nblk=NB):
        if isinstance(j, int):
            lr = slice(j * 128, (j + 1) * 128)
            li = slice(P + j * 128, P + (j + 1) * 128)
        else:
            lr = pl.ds(pl.multiple_of(j * 128, 128), 128)
            li = pl.ds(pl.multiple_of(P + j * 128, 128), 128)
        tabs = [tab_ref[n, :, lr] for n in range(10)]
        cr = carry_ref[0, :, lr]
        ci = carry_ref[1, :, lr]
        for kb in range(nblk):
            if isinstance(row0, int):
                rows = slice(row0 + kb * 8, row0 + kb * 8 + 8)
            else:
                rows = pl.ds(pl.multiple_of(row0 + kb * 8, 8), 8)
            hr, hi = _cmul(tabs[0], tabs[1], h_ref[rows, lr], h_ref[rows, li])
            for n, s in enumerate((1, 2, 4)):
                sr = pltpu.roll(hr, s, 0)
                si = pltpu.roll(hi, s, 0)
                dr, di = _cmul(tabs[2 + 2 * n], tabs[3 + 2 * n], sr, si)
                hr = hr + dr
                hi = hi + di
            dr, di = _cmul(tabs[8], tabs[9], cr, ci)
            hr = hr + dr
            hi = hi + di
            cr = jnp.broadcast_to(hr[7:8, :], (8, 128))
            ci = jnp.broadcast_to(hi[7:8, :], (8, 128))
            h_ref[rows, lr] = hr * 2.0
            h_ref[rows, li] = hi * (-2.0)
        carry_ref[0, :, lr] = cr
        carry_ref[1, :, lr] = ci

    scan_group(NGRP - 1, 0, 1)

    def ffn_body(c, _):
        @pl.when(step == 0)
        def _wait():
            for cp in ffn_copies(c):
                cp.wait()

            @pl.when(c + 2 < NF)
            def _start_next():
                for cp in ffn_copies(jnp.minimum(c + 2, NF - 1)):
                    cp.start()

            @pl.when(c + 2 == NF)
            def _start_c():
                for cp in c_copies():
                    cp.start()
        cs = pl.ds(pl.multiple_of(c * FC, FC), FC)
        g = jnp.dot(x_ref[...], wg_ref[:, cs], preferred_element_type=f32).astype(bf16).astype(f32)
        u = jnp.dot(x_ref[...], wu_ref[:, cs], preferred_element_type=f32).astype(bf16).astype(f32)
        hh = (_gelu_tanh(g).astype(bf16).astype(f32) * u).astype(bf16)
        part = jnp.dot(hh, wd_ref[cs, :], preferred_element_type=f32)
        acc_ref[...] += part
        scan_group(c)
        scan_group(NGRP - 1, 8 + c * (8 * XB), XB)
        return 0
    jax.lax.fori_loop(0, NF, ffn_body, 0)

    @pl.when(step == 0)
    def _wait_c():
        for cp in c_copies():
            cp.wait()

    gf = gate_ref[:, 0:1]
    omg = (1.0 - gf).astype(bf16)

    @pl.when(step >= 2)
    def _drain():
        for n in range(NOC):
            out_copy(jnp.maximum(step - 2, 0), n).wait()

    hre = h_ref[:, :P].astype(bf16)
    him = h_ref[:, P:].astype(bf16)
    dsk = dsk_ref[...].reshape(1, D)
    for n in range(NOC):
        cols = slice(n * OC, (n + 1) * OC)
        ya = (jax.lax.dot_general(hre, cre_ref[cols, :], NT_DIMS, preferred_element_type=f32)
              + jax.lax.dot_general(him, cim_ref[cols, :], NT_DIMS, preferred_element_type=f32))
        ya = ya + (x_ref[:, cols] * dsk[:, cols]).astype(f32)
        yb = acc_ref[:, cols].astype(bf16)
        obuf_ref[step % 2, :, cols] = gf * ya + (omg * yb).astype(f32)
        out_copy(step, n).start()

    @pl.when(step == L // T - 1)
    def _finish():
        for n in range(NOC):
            out_copy(jnp.maximum(step - 1, 0), n).wait()
        for n in range(NOC):
            out_copy(step, n).wait()


@jax.jit
def pallas_gated_mix__ssm_conv_s5__glu_gated_geglu__prompt_kernel(
    A_x, A_Lambda_re, A_Lambda_im, A_B_re, A_B_im, A_C_re, A_C_im, A_log_dt, A_Dskip,
    B_x, B_w_gate, B_w_up, B_w_down, gate_w,
):
    x2 = A_x.reshape(L, D)
    const = lambda shape: pl.BlockSpec(shape, lambda i: (0,))
    hbm = pl.BlockSpec(memory_space=pl.ANY)
    out = pl.pallas_call(
        _kernel,
        grid=(L // T,),
        in_specs=[
            pl.BlockSpec((T, D), lambda i: (i, 0)),
            const((P,)), const((P,)), const((P,)), const((D,)), const((D,)),
            hbm, hbm, hbm, hbm, hbm, hbm, hbm,
        ],
        out_specs=pl.BlockSpec(memory_space=pl.ANY),
        out_shape=jax.ShapeDtypeStruct((L, D), jnp.float32),
        scratch_shapes=[
            pltpu.VMEM((P, D), jnp.bfloat16),
            pltpu.VMEM((P, D), jnp.bfloat16),
            pltpu.VMEM((D, P), jnp.bfloat16),
            pltpu.VMEM((D, P), jnp.bfloat16),
            pltpu.VMEM((D, DF), jnp.bfloat16),
            pltpu.VMEM((D, DF), jnp.bfloat16),
            pltpu.VMEM((DF, D), jnp.bfloat16),
            pltpu.VMEM((10, 8, P), jnp.float32),
            pltpu.VMEM((2, 8, P), jnp.float32),
            pltpu.VMEM((T, 2 * P), jnp.float32),
            pltpu.VMEM((T, D), jnp.float32),
            pltpu.VMEM((2, T, D), jnp.float32),
            pltpu.VMEM((T, 128), jnp.float32),
            pltpu.SemaphoreType.DMA((2 + 3 * NF,)),
            pltpu.SemaphoreType.DMA((2, NOC)),
            pltpu.SemaphoreType.DMA((2 * NBC,)),
        ],
        compiler_params=pltpu.CompilerParams(
            dimension_semantics=("arbitrary",),
            vmem_limit_bytes=110 * 1024 * 1024,
        ),
    )(x2, A_Lambda_re, A_Lambda_im, A_log_dt, A_Dskip, gate_w,
      A_B_re, A_B_im, A_C_re, A_C_im, B_w_gate, B_w_up, B_w_down)
    return out.reshape(1, L, D)
```
